```python
import os as _os
_os.environ.setdefault("JAX_PLATFORMS", "cpu")
import jax
import jax.numpy as jnp

def _softmax(x, axis=-1):
    return jax.nn.softmax(x, axis=axis)
def _gelu(x):
    return jax.nn.gelu(x, approximate=True)
def _silu(x):
    return jax.nn.silu(x)
def _sigmoid(x):
    return jax.nn.sigmoid(x)
def _layernorm(x, axis=-1, eps=1e-5):
    m = jnp.mean(x, axis=axis, keepdims=True)
    v = jnp.var(x, axis=axis, keepdims=True)
    return (x - m) / jnp.sqrt(v + eps)
def _scatter_add(tgt, idx, src, axis=0):
    return tgt.at[idx].add(src)
def _segment_sum(src, seg, n):
    return jax.ops.segment_sum(src, seg, n)
class _Rng:
    def __init__(self, key):
        self._k = key
    def _next(self):
        self._k, sub = jax.random.split(self._k)
        return sub
    def normal(self, shape):
        return jax.random.normal(self._next(), shape, dtype=jnp.bfloat16)
    def randint(self, lo, hi, shape):
        return jax.random.randint(self._next(), shape, lo, hi, dtype=jnp.int32)
    def uniform(self, shape, lo=0.0, hi=1.0):
        return jax.random.uniform(self._next(), shape, jnp.bfloat16, lo, hi)
    def permutation(self, n):
        return jax.random.permutation(self._next(), n)


kernel_name = 'sequential_preLN__compressed_kv_cla__dense_activation_mish__decode'

def setup_inputs():
    _rng = _Rng(jax.random.key(int.from_bytes(__import__("os").urandom(4), "little")))
    _w = (lambda a: (lambda t: t.astype(jnp.bfloat16) if jnp.issubdtype(t.dtype, jnp.floating) else t)(jnp.asarray(a)))
    def _A_setup():
        B, H, Sq, Sk, D, M = 2, 32, 1, 8192, 128, 512
        Dc = 4 * D
        return {
            "x": _w((lambda *s: _rng.normal(s) * 0.05)(B, Sq, M)),
            "c_kv": _w((lambda *s: _rng.normal(s) * 0.8)(B, Sk, Dc)),
            "w_q": _w((lambda *s: _rng.normal(s) * 0.8)(M, H, D) * (M ** -0.5)),
            "w_uk": _w((lambda *s: _rng.normal(s) * 0.8)(Dc, H, D) * (Dc ** -0.5)),
            "w_uv": _w((lambda *s: _rng.normal(s) * 0.8)(Dc, H, D) * (Dc ** -0.5)),
            "w_o": _w((lambda *s: _rng.normal(s) * 0.8)(H, D, M) * ((H * D) ** -0.5)),
        }
    _A_in = _A_setup()

    def _B_setup():
        B, S, D, F = 2, 1, 512, 1792
        return {
            "x": _w((lambda *s: _rng.normal(s) * 0.05)(B, S, D)),
            "w1": _w((lambda *s: _rng.normal(s) * 0.4)(D, F) * (D ** -0.5)),
            "b1": _w((lambda *s: _rng.normal(s) * 0.05)(F)),
            "w2": _w((lambda *s: _rng.normal(s) * 0.05)(F, D) * (F ** -0.5)),
        }
    _B_in = _B_setup()

    return {
        "A_x": _A_in["x"],
        "A_c_kv": _A_in["c_kv"],
        "A_w_q": _A_in["w_q"],
        "A_w_uk": _A_in["w_uk"],
        "A_w_uv": _A_in["w_uv"],
        "A_w_o": _A_in["w_o"],
        "B_x": _B_in["x"],
        "B_w1": _B_in["w1"],
        "B_b1": _B_in["b1"],
        "B_w2": _B_in["w2"],
    }

def reference(A_x, A_c_kv, A_w_q, A_w_uk, A_w_uv, A_w_o, B_x, B_w1, B_b1, B_w2):
    def _A_ref(x, c_kv, w_q, w_uk, w_uv, w_o):
        B, Sq, M = x.shape[0], x.shape[1], x.shape[2]
        Sk = c_kv.shape[1]
        H, D = w_q.shape[1], w_q.shape[2]
        q = jnp.einsum("bqm,mhd->bhqd", x, w_q)
        k = jnp.einsum("bkc,chd->bhkd", c_kv, w_uk)
        v = jnp.einsum("bkc,chd->bhkd", c_kv, w_uv)
        scores = jnp.einsum("bhqd,bhkd->bhqk", q, k) * (D ** -0.5)
        off = Sk - Sq
        qi = jnp.arange(Sq)[:, None]
        kj = jnp.arange(Sk)[None, :]
        cmask = kj <= (qi + off)
        scores = jnp.where(cmask[None, None], scores, -1e9)
        p = _softmax(scores, axis=-1)
        ctx = jnp.einsum("bhqk,bhkd->bhqd", p, v)
        return jnp.einsum("bhqd,hdm->bqm", ctx, w_o)

    def _B_ref(x, w1, b1, w2):
        h = jnp.einsum("bsd,df->bsf", x, w1) + b1
        sp = jnp.log1p(jnp.exp(-jnp.abs(h))) + jnp.where(h > 0, h, jnp.zeros_like(h))
        act = h * jnp.tanh(sp)
        return jnp.einsum("bsf,fd->bsd", act, w2)

    x = A_x
    h = x + _A_ref(_layernorm(x, axis=-1), A_c_kv, A_w_q, A_w_uk, A_w_uv, A_w_o)
    h2 = h + _B_ref(_layernorm(h, axis=-1), B_w1, B_b1, B_w2)
    return h2
```

```python
import functools
import jax
import jax.numpy as jnp
from jax import lax
import jax.experimental.pallas as pl
import jax.experimental.pallas.tpu as pltpu

B, H, D, M, DC, SK, F = 2, 32, 128, 512, 512, 8192, 1792
F32, BF16 = jnp.float32, jnp.bfloat16
NT = (((1,), (1,)), ((), ()))


def _ln(x):
    m = jnp.mean(x, axis=-1, keepdims=True)
    xc = x - m
    v = jnp.mean(xc * xc, axis=-1, keepdims=True)
    return xc / jnp.sqrt(v + 1e-5)


def _rows16(x2):
    n = x2.shape[-1]
    return jnp.concatenate([jnp.broadcast_to(x2[0:1], (8, n)), jnp.broadcast_to(x2[1:2], (8, n))], axis=0)


def make_kernel(CKC=1024, SUB=512, NSEM=4, ALL_UP=False):
    NCK = SK // CKC

    def kernel(x_ref, b1_ref, ckv_h, wq_h, wuk_h, wuv_h, wo_h, w1_h, w2_h, out_ref,
               ckv_v, wq_v, wuk_v, wuv_v, wo_v, w1_v, w2_v, s_v, sems):
        copies = []
        def add(src, dst, n, rows):
            r = rows // n
            for i in range(n):
                copies.append((src.at[pl.ds(i * r, r)], dst.at[pl.ds(i * r, r)]))
        add(wq_h, wq_v, 4, 16384)
        add(wuk_h, wuk_v, 4, 16384)
        add(ckv_h, ckv_v, B * NCK, B * SK)
        add(wuv_h, wuv_v, 4, 16384)
        add(wo_h, wo_v, 4, 4096)
        add(w1_h, w1_v, 4, 512)
        add(w2_h, w2_v, 4, 1792)
        ncp = len(copies)
        nsem = ncp if ALL_UP else NSEM
        descs = [pltpu.make_async_copy(s, d, sems.at[i % nsem]) for i, (s, d) in enumerate(copies)]
        for i in range(min(nsem, ncp)):
            descs[i].start()
        state = {"n": 0}
        def wait_next():
            n = state["n"]
            descs[n].wait()
            if n + nsem < ncp:
                descs[n + nsem].start()
            state["n"] = n + 1

        row16 = lax.broadcasted_iota(jnp.int32, (16, 256), 0)
        lane16 = lax.broadcasted_iota(jnp.int32, (16, 256), 1)
        j16 = row16 % 8
        par16 = lane16 % 2
        e_r = lax.broadcasted_iota(jnp.int32, (128, 256), 0)
        e_l = lax.broadcasted_iota(jnp.int32, (128, 256), 1)
        E2 = jnp.where(e_l // 2 == e_r, 1.0, 0.0).astype(BF16)
        c_r = lax.broadcasted_iota(jnp.int32, (256, 128), 0)
        c_l = lax.broadcasted_iota(jnp.int32, (256, 128), 1)
        C2 = jnp.where(c_r // 2 == c_l, 1.0, 0.0).astype(BF16)
        j128 = lax.broadcasted_iota(jnp.int32, (16, 128), 0) % 8

        def expand_masked(a_blk):
            xe = jnp.dot(a_blk, E2, preferred_element_type=F32)
            return jnp.concatenate(
                [jnp.where(par16 + 2 * ii == j16, xe, 0.0).astype(BF16) for ii in range(4)], axis=1)

        def wpair(w_v, cc, i):
            wu = w_v.bitcast(jnp.uint32)
            return pltpu.bitcast(wu[pl.ds(16 * 128 * cc + i, 128, stride=16), :], BF16)

        x = x_ref[...].astype(F32)
        xn16 = _rows16(_ln(x)).astype(BF16)

        q = [jnp.zeros((16, 128), F32) for _ in range(4)]
        for cc in range(4):
            lhs = expand_masked(xn16[:, 128 * cc:128 * (cc + 1)])
            wait_next()
            for g in range(4):
                rhs = jnp.concatenate([wpair(wq_v, cc, 4 * g + ii) for ii in range(4)], axis=0)
                q[g] = q[g] + jnp.dot(lhs, rhs, preferred_element_type=F32)
        scale = D ** -0.5
        qm = []
        for g in range(4):
            qb = (q[g] * scale).astype(BF16)
            qm.append(jnp.concatenate([jnp.where(j128 // 2 == ii, qb, jnp.zeros_like(qb)) for ii in range(4)], axis=1))

        qabs = [[None] * 4 for _ in range(4)]
        for cc in range(4):
            wait_next()
            for g in range(4):
                rhs = jnp.concatenate([wpair(wuk_v, cc, 4 * g + ii) for ii in range(4)], axis=1)
                y = lax.dot_general(qm[g], rhs, NT, preferred_element_type=F32)
                y = jnp.where(par16 == j16 % 2, y, 0.0).astype(BF16)
                qabs[g][cc] = jnp.dot(y, C2, preferred_element_type=F32)
        qa = []
        for b in range(B):
            qa.append(jnp.concatenate(
                [jnp.concatenate([qabs[g][cc][8 * b:8 * b + 8] for cc in range(4)], axis=1) for g in range(4)],
                axis=0).astype(BF16))

        ctxc = []
        for b in range(B):
            mrun = jnp.full((H, 128), -jnp.inf, F32)
            for ch in range(NCK):
                wait_next()
                def s_body(t, mrun, ch=ch, b=b):
                    off = pl.multiple_of(ch * CKC + t * SUB, SUB)
                    kv = ckv_v[pl.ds(b * SK + off, SUB), :]
                    s = lax.dot_general(qa[b], kv, NT, preferred_element_type=F32)
                    s_v[b, :, pl.ds(off, SUB)] = s
                    for u in range(SUB // 128):
                        mrun = jnp.maximum(mrun, s[:, 128 * u:128 * (u + 1)])
                    return mrun
                mrun = lax.fori_loop(0, CKC // SUB, s_body, mrun)
            m = jnp.max(mrun, axis=1, keepdims=True)
            def pv_body(t, carry, b=b, m=m):
                acc, lrun = carry
                off = pl.multiple_of(t * SUB, SUB)
                p = jnp.exp(s_v[b, :, pl.ds(off, SUB)] - m)
                for u in range(SUB // 128):
                    lrun = lrun + p[:, 128 * u:128 * (u + 1)]
                kv = ckv_v[pl.ds(b * SK + off, SUB), :]
                acc = acc + jnp.dot(p.astype(BF16), kv, preferred_element_type=F32)
                return acc, lrun
            acc, lrun = lax.fori_loop(0, SK // SUB, pv_body,
                                      (jnp.zeros((H, DC), F32), jnp.zeros((H, 128), F32)))
            l = jnp.sum(lrun, axis=1, keepdims=True)
            ctxc.append(acc / l)

        ctx = [jnp.zeros((16, 128), F32) for _ in range(4)]
        cg = [jnp.concatenate([ctxc[0][8 * g:8 * g + 8], ctxc[1][8 * g:8 * g + 8]], axis=0).astype(BF16) for g in range(4)]
        for cc in range(4):
            lhs = [expand_masked(cg[g][:, 128 * cc:128 * (cc + 1)]) for g in range(4)]
            wait_next()
            for g in range(4):
                rhs = jnp.concatenate([wpair(wuv_v, cc, 4 * g + ii) for ii in range(4)], axis=0)
                ctx[g] = ctx[g] + jnp.dot(lhs[g], rhs, preferred_element_type=F32)

        acc = jnp.zeros((16, M), F32)
        for g in range(4):
            cb = ctx[g].astype(BF16)
            lhs = jnp.concatenate([jnp.where(j128 == j, cb, jnp.zeros_like(cb)) for j in range(8)], axis=1)
            wait_next()
            acc = acc + jnp.dot(lhs, wo_v[pl.ds(1024 * g, 1024), :], preferred_element_type=F32)
        att = jnp.concatenate([jnp.sum(acc[0:8], axis=0, keepdims=True), jnp.sum(acc[8:16], axis=0, keepdims=True)], axis=0)
        h = x + att
        hn16 = _rows16(_ln(h)).astype(BF16)

        t = jnp.zeros((16, F), F32)
        for kk in range(4):
            wait_next()
            t = t + jnp.dot(hn16[:, 128 * kk:128 * (kk + 1)], w1_v[pl.ds(128 * kk, 128), :], preferred_element_type=F32)
        t = jnp.concatenate([t[0:1], t[8:9]], axis=0) + b1_ref[...].reshape(1, F).astype(F32)
        sp = jnp.log1p(jnp.exp(-jnp.abs(t))) + jnp.maximum(t, 0.0)
        act16 = _rows16(t * jnp.tanh(sp)).astype(BF16)
        o = jnp.zeros((16, M), F32)
        R2 = F // 4
        for kk in range(4):
            wait_next()
            o = o + jnp.dot(act16[:, R2 * kk:R2 * (kk + 1)], w2_v[pl.ds(R2 * kk, R2), :], preferred_element_type=F32)
        out = h + jnp.concatenate([o[0:1], o[8:9]], axis=0)
        out_ref[...] = out.astype(out_ref.dtype)

    @jax.jit
    def fn(A_x, A_c_kv, A_w_q, A_w_uk, A_w_uv, A_w_o, B_x, B_w1, B_b1, B_w2):
        del B_x
        nsem = (4 + 4 + B * NCK + 4 + 4 + 4 + 4) if ALL_UP else NSEM
        any_spec = pl.BlockSpec(memory_space=pl.ANY)
        vm = pl.BlockSpec(memory_space=pltpu.VMEM)
        out = pl.pallas_call(
            kernel,
            out_shape=jax.ShapeDtypeStruct((B, M), A_x.dtype),
            in_specs=[vm, vm] + [any_spec] * 7,
            out_specs=vm,
            scratch_shapes=[
                pltpu.VMEM((B * SK, DC), BF16),
                pltpu.VMEM((M * H, D), BF16), pltpu.VMEM((DC * H, D), BF16), pltpu.VMEM((DC * H, D), BF16),
                pltpu.VMEM((H * D, M), BF16), pltpu.VMEM((M, F), BF16), pltpu.VMEM((F, M), BF16),
                pltpu.VMEM((B, H, SK), F32),
                pltpu.SemaphoreType.DMA((nsem,)),
            ],
            compiler_params=pltpu.CompilerParams(vmem_limit_bytes=64 * 1024 * 1024),
        )(A_x.reshape(B, M), B_b1, A_c_kv.reshape(B * SK, DC), A_w_q.reshape(M * H, D),
          A_w_uk.reshape(DC * H, D), A_w_uv.reshape(DC * H, D), A_w_o.reshape(H * D, M), B_w1, B_w2)
        return out.reshape(B, 1, M)
    return fn


pallas_sequential_preLN__compressed_kv_cla__dense_activation_mish__decode_kernel = make_kernel()
```

```python
import jax
import jax.numpy as jnp
from jax import lax
import jax.experimental.pallas as pl
import jax.experimental.pallas.tpu as pltpu

B, H, D, M, DC, SK, F = 2, 32, 128, 512, 512, 8192, 1792
F32, BF16 = jnp.float32, jnp.bfloat16
NT = (((1,), (1,)), ((), ()))

SUB = 512
NS = SK // SUB
NSEM = 5
PIECE_BYTES = 40 * 1024
PATTERN = (1, 1, 0)
W1_CHUNKS = (128, 128, 128, 128)
W2_CHUNKS = (512, 512, 512, 256)


def _ln(x):
    m = jnp.mean(x, axis=-1, keepdims=True)
    xc = x - m
    v = jnp.mean(xc * xc, axis=-1, keepdims=True)
    return xc / jnp.sqrt(v + 1e-5)


def _rows16(x2):
    n = x2.shape[-1]
    return jnp.concatenate(
        [jnp.broadcast_to(x2[0:1], (8, n)), jnp.broadcast_to(x2[1:2], (8, n))], axis=0)


def _row_lane_ids():
    row = lax.broadcasted_iota(jnp.int32, (16, 256), 0)
    lane = lax.broadcasted_iota(jnp.int32, (16, 256), 1)
    return row % 8, lane % 2


def _expand_matrix():
    r = lax.broadcasted_iota(jnp.int32, (128, 256), 0)
    l = lax.broadcasted_iota(jnp.int32, (128, 256), 1)
    return jnp.where(l // 2 == r, 1.0, 0.0).astype(BF16)


def _expand_masked(a_blk, e2, j16, par16):
    xe = jnp.dot(a_blk, e2, preferred_element_type=F32)
    return jnp.concatenate(
        [jnp.where(par16 + 2 * ii == j16, xe, 0.0).astype(BF16) for ii in range(4)], axis=1)


def _head_pair(w_v, cc, i):
    wu = w_v.bitcast(jnp.uint32)
    return pltpu.bitcast(wu[pl.ds(16 * 128 * cc + i, 128, stride=16), :], BF16)


def _kernel(x_h, b1_h, ckv_h, wq_h, wuk_h, wuv_h, wo_h, w1_h, w2_h, out_ref,
            ckv_v, wq_v, wuk_v, wuv_v, wo_v, w1_v, w2_v, s_v, x_v, b1_v, sems):
    chunks = []

    def add(src, dst, splits, piece_rows):
        o = 0
        for r in splits:
            chunks.append((src, dst, o, r, piece_rows))
            o += r
        assert o == src.shape[0]

    p128 = PIECE_BYTES // (128 * 2)
    p512 = PIECE_BYTES // (512 * 2)
    add(wq_h, wq_v, (2048,) * 8, p128)
    add(wuk_h, wuk_v, (2048,) * 8, p128)
    add(ckv_h, ckv_v, (SUB,) * (B * NS), p512)
    add(wuv_h, wuv_v, (2048,) * 8, p128)
    add(wo_h, wo_v, (512,) * 8, p512)
    add(w1_h, w1_v, W1_CHUNKS, 8)
    add(w2_h, w2_v, W2_CHUNKS, p512)
    n_chunks = len(chunks)
    st = {"piece": 0, "n": 0}

    def start_chunk(n):
        src, dst, o, r, piece_rows = chunks[n]
        sem = sems.at[n % NSEM]
        npc = max(1, round(r / piece_rows))
        units = r // 8
        for j in range(npc):
            sz = 8 * (units // npc + (1 if j < units % npc else 0))
            pltpu.make_async_copy(src.at[pl.ds(o, sz)], dst.at[pl.ds(o, sz)], sem).start(
                priority=PATTERN[st["piece"] % len(PATTERN)])
            st["piece"] += 1
            o += sz
        assert o == chunks[n][2] + r

    cx = pltpu.make_async_copy(x_h, x_v, sems.at[0])
    cb = pltpu.make_async_copy(b1_h, b1_v, sems.at[0])
    cx.start()
    cb.start()
    for n in range(NSEM):
        start_chunk(n)

    def wait_next():
        n = st["n"]
        src, dst, o, r, _ = chunks[n]
        whole = dst.at[pl.ds(o, r)]
        pltpu.make_async_copy(whole, whole, sems.at[n % NSEM]).wait()
        if n == 0:
            cx.wait()
            cb.wait()
        if n + NSEM < n_chunks:
            start_chunk(n + NSEM)
        st["n"] = n + 1

    wait_next()
    x = x_v[...].astype(F32)
    xn16 = _rows16(_ln(x)).astype(BF16)
    j16, par16 = _row_lane_ids()
    e2 = _expand_matrix()
    q = [jnp.zeros((16, D), F32) for _ in range(4)]
    for cc in range(4):
        lhs = _expand_masked(xn16[:, 128 * cc:128 * (cc + 1)], e2, j16, par16)
        for w in range(2):
            if cc + w > 0:
                wait_next()
        for g in range(4):
            rhs = jnp.concatenate([_head_pair(wq_v, cc, 4 * g + ii) for ii in range(4)], axis=0)
            q[g] = q[g] + jnp.dot(lhs, rhs, preferred_element_type=F32)
    j128 = lax.broadcasted_iota(jnp.int32, (16, 128), 0) % 8
    qm = []
    for g in range(4):
        qb = (q[g] * (D ** -0.5)).astype(BF16)
        qm.append(jnp.concatenate(
            [jnp.where(j128 // 2 == ii, qb, jnp.zeros_like(qb)) for ii in range(4)], axis=1))

    c_r = lax.broadcasted_iota(jnp.int32, (256, 128), 0)
    c_l = lax.broadcasted_iota(jnp.int32, (256, 128), 1)
    c2 = jnp.where(c_r // 2 == c_l, 1.0, 0.0).astype(BF16)
    qabs = [[None] * 4 for _ in range(4)]
    for cc in range(4):
        wait_next()
        wait_next()
        for g in range(4):
            rhs = jnp.concatenate([_head_pair(wuk_v, cc, 4 * g + ii) for ii in range(4)], axis=1)
            y = lax.dot_general(qm[g], rhs, NT, preferred_element_type=F32)
            y = jnp.where(par16 == j16 % 2, y, 0.0).astype(BF16)
            qabs[g][cc] = jnp.dot(y, c2, preferred_element_type=F32)
    qa = []
    for b in range(B):
        qa.append(jnp.concatenate(
            [jnp.concatenate([qabs[g][cc][8 * b:8 * b + 8] for cc in range(4)], axis=1)
             for g in range(4)], axis=0).astype(BF16))

    def scores(b, t, mrun):
        kv = ckv_v[pl.ds(b * SK + t * SUB, SUB), :]
        s = lax.dot_general(qa[b], kv, NT, preferred_element_type=F32)
        s_v[b, :, pl.ds(t * SUB, SUB)] = s
        for u in range(SUB // 128):
            mrun = jnp.maximum(mrun, s[:, 128 * u:128 * (u + 1)])
        return mrun

    def pv(b, t, m, acc, lrun):
        p = jnp.exp(s_v[b, :, pl.ds(t * SUB, SUB)] - m)
        for u in range(SUB // 128):
            lrun = lrun + p[:, 128 * u:128 * (u + 1)]
        kv = ckv_v[pl.ds(b * SK + t * SUB, SUB), :]
        return acc + jnp.dot(p.astype(BF16), kv, preferred_element_type=F32), lrun

    neg = jnp.full((H, 128), -jnp.inf, F32)
    mrun = neg
    for t in range(NS):
        wait_next()
        mrun = scores(0, t, mrun)
    m0 = jnp.max(mrun, axis=1, keepdims=True)
    mrun = neg
    acc, lrun = jnp.zeros((H, DC), F32), jnp.zeros((H, 128), F32)
    for t in range(NS):
        wait_next()
        mrun = scores(1, t, mrun)
        acc, lrun = pv(0, t, m0, acc, lrun)
    m1 = jnp.max(mrun, axis=1, keepdims=True)
    ctxc = [acc / jnp.sum(lrun, axis=1, keepdims=True)]
    acc, lrun = jnp.zeros((H, DC), F32), jnp.zeros((H, 128), F32)
    for t in range(NS):
        if t % 2 == 0:
            wait_next()
        acc, lrun = pv(1, t, m1, acc, lrun)
    ctxc.append(acc / jnp.sum(lrun, axis=1, keepdims=True))

    j16, par16 = _row_lane_ids()
    e2 = _expand_matrix()
    ctx = [jnp.zeros((16, D), F32) for _ in range(4)]
    cg = [jnp.concatenate([ctxc[0][8 * g:8 * g + 8], ctxc[1][8 * g:8 * g + 8]], axis=0).astype(BF16)
          for g in range(4)]
    for cc in range(4):
        lhs = [_expand_masked(cg[g][:, 128 * cc:128 * (cc + 1)], e2, j16, par16) for g in range(4)]
        for g in range(4):
            if g % 2 == 0:
                wait_next()
            rhs = jnp.concatenate([_head_pair(wuv_v, cc, 4 * g + ii) for ii in range(4)], axis=0)
            ctx[g] = ctx[g] + jnp.dot(lhs[g], rhs, preferred_element_type=F32)

    j128 = lax.broadcasted_iota(jnp.int32, (16, 128), 0) % 8
    acc = jnp.zeros((16, M), F32)
    for g in range(4):
        cbf = ctx[g].astype(BF16)
        lhs = jnp.concatenate(
            [jnp.where(j128 == j, cbf, jnp.zeros_like(cbf)) for j in range(8)], axis=1)
        wait_next()
        acc = acc + jnp.dot(lhs, wo_v[pl.ds(1024 * g, 1024), :], preferred_element_type=F32)
    att = jnp.concatenate([jnp.sum(acc[0:8], axis=0, keepdims=True),
                           jnp.sum(acc[8:16], axis=0, keepdims=True)], axis=0)
    h = x + att
    hn = _ln(h)
    r16 = lax.broadcasted_iota(jnp.int32, (16, M), 0)
    hn16 = jnp.where(r16 == 0, jnp.broadcast_to(hn[0:1], (16, M)),
                     jnp.where(r16 == 1, jnp.broadcast_to(hn[1:2], (16, M)), 0.0)).astype(BF16)

    t1 = jnp.zeros((8, F), F32)
    for kk in range(4):
        t1 = t1 + jnp.dot(hn16[:, 128 * kk:128 * (kk + 1)], w1_v[pl.ds(128 * kk, 128), :],
                          preferred_element_type=F32)[0:8]
    t1 = t1 + b1_v[...].reshape(1, F).astype(F32)
    sp = jnp.log1p(jnp.exp(-jnp.abs(t1))) + jnp.maximum(t1, 0.0)
    act = t1 * jnp.tanh(sp)
    act16 = jnp.concatenate([act, jnp.zeros((8, F), F32)], axis=0).astype(BF16)
    o = jnp.zeros((8, M), F32)
    off = 0
    for r in W2_CHUNKS:
        wait_next()
        o = o + jnp.dot(act16[:, off:off + r], w2_v[pl.ds(off, r), :],
                        preferred_element_type=F32)[0:8]
        off += r
    assert st["n"] == n_chunks
    out_ref[...] = (h + o[0:2]).astype(out_ref.dtype)


@jax.jit
def pallas_sequential_preLN__compressed_kv_cla__dense_activation_mish__decode_kernel(
    A_x: jax.Array,
    A_c_kv: jax.Array,
    A_w_q: jax.Array,
    A_w_uk: jax.Array,
    A_w_uv: jax.Array,
    A_w_o: jax.Array,
    B_x: jax.Array,
    B_w1: jax.Array,
    B_b1: jax.Array,
    B_w2: jax.Array,
):
    del B_x
    any_spec = pl.BlockSpec(memory_space=pl.ANY)
    out = pl.pallas_call(
        _kernel,
        out_shape=jax.ShapeDtypeStruct((B, M), A_x.dtype),
        in_specs=[any_spec] * 9,
        out_specs=pl.BlockSpec(memory_space=pltpu.VMEM),
        scratch_shapes=[
            pltpu.VMEM((B * SK, DC), BF16),
            pltpu.VMEM((M * H, D), BF16),
            pltpu.VMEM((DC * H, D), BF16),
            pltpu.VMEM((DC * H, D), BF16),
            pltpu.VMEM((H * D, M), BF16),
            pltpu.VMEM((M, F), BF16),
            pltpu.VMEM((F, M), BF16),
            pltpu.VMEM((B, H, SK), F32),
            pltpu.VMEM((B, M), BF16),
            pltpu.VMEM((F,), BF16),
            pltpu.SemaphoreType.DMA((NSEM,)),
        ],
        compiler_params=pltpu.CompilerParams(vmem_limit_bytes=64 * 1024 * 1024),
    )(A_x.reshape(B, M), B_b1, A_c_kv.reshape(B * SK, DC), A_w_q.reshape(M * H, D),
      A_w_uk.reshape(DC * H, D), A_w_uv.reshape(DC * H, D), A_w_o.reshape(H * D, M), B_w1, B_w2)
    return out.reshape(B, 1, M)
```

```python
import jax
import jax.numpy as jnp
from jax import lax
import jax.experimental.pallas as pl
import jax.experimental.pallas.tpu as pltpu

B, H, D, M, DC, SK, F = 2, 32, 128, 512, 512, 8192, 1792
F32, BF16 = jnp.float32, jnp.bfloat16
NT = (((1,), (1,)), ((), ()))

SUB = 512
NS = SK // SUB
NSEM = 5
PIECE_BYTES = 32 * 1024
LOW_SHARE = 5 / 16
PAD = 32
W1_CHUNKS = (128, 128, 128, 128)
W2_CHUNKS = (512, 512, 512, 256)


def _ln(x):
    m = jnp.mean(x, axis=-1, keepdims=True)
    xc = x - m
    v = jnp.mean(xc * xc, axis=-1, keepdims=True)
    return xc / jnp.sqrt(v + 1e-5)


def _rows16(x2):
    n = x2.shape[-1]
    return jnp.concatenate(
        [jnp.broadcast_to(x2[0:1], (8, n)), jnp.broadcast_to(x2[1:2], (8, n))], axis=0)


def _row_lane_ids():
    row = lax.broadcasted_iota(jnp.int32, (16, 256), 0)
    lane = lax.broadcasted_iota(jnp.int32, (16, 256), 1)
    return row % 8, lane % 2


def _expand_matrix():
    r = lax.broadcasted_iota(jnp.int32, (128, 256), 0)
    l = lax.broadcasted_iota(jnp.int32, (128, 256), 1)
    return jnp.where(l // 2 == r, 1.0, 0.0).astype(BF16)


def _expand_masked(a_blk, e2, j16, par16):
    xe = jnp.dot(a_blk, e2, preferred_element_type=F32)
    return jnp.concatenate(
        [jnp.where(par16 + 2 * ii == j16, xe, 0.0).astype(BF16) for ii in range(4)], axis=1)


def _head_pair(w_v, cc, i):
    wu = w_v.bitcast(jnp.uint32)
    return pltpu.bitcast(wu[pl.ds(16 * 128 * cc + i, 128, stride=16), :], BF16)


def _kernel(x_h, b1_h, ckv_h, wq_h, wuk_h, wuv_h, wo_h, w1_h, w2_h, out_ref,
            ckv_v, wq_v, wuk_v, wuv_v, wo_v, w1_v, w2_v, s_v, x_v, b1_v, sems):
    chunks = []

    def add(src, dst, splits, piece_rows):
        o = 0
        for r in splits:
            chunks.append((src, dst, o, r, piece_rows))
            o += r
        assert o == src.shape[0] <= dst.shape[0]

    p128 = PIECE_BYTES // (128 * 2)
    p512 = PIECE_BYTES // (512 * 2)
    add(wq_h, wq_v, (2048,) * 8, p128)
    add(wuk_h, wuk_v, (2048,) * 8, p128)
    add(ckv_h, ckv_v, (SUB,) * (B * NS), p512)
    add(wuv_h, wuv_v, (2048,) * 8, p128)
    add(wo_h, wo_v, (512,) * 8, p512)
    add(w1_h, w1_v, W1_CHUNKS, 8)
    add(w2_h, w2_v, W2_CHUNKS, p512)
    n_chunks = len(chunks)
    st = {"n": 0}

    def pieces(o, r, piece_rows):
        npc = max(1, round(r / piece_rows))
        units = r // 8
        out = []
        for j in range(npc):
            sz = 8 * (units // npc + (1 if j < units % npc else 0))
            out.append((o, sz))
            o += sz
        return out

    def start_chunk(n):
        src, dst, o, r, piece_rows = chunks[n]
        sem = sems.at[n % NSEM]
        r0 = 8 * max(1, round(r * LOW_SHARE / 8))
        lo, hi = pieces(o, r0, piece_rows), pieces(o + r0, r - r0, piece_rows)
        i0 = i1 = 0
        while i0 < len(lo) or i1 < len(hi):
            if i1 >= len(hi) or (i0 < len(lo) and i0 * len(hi) <= i1 * len(lo)):
                (po, sz), priority = lo[i0], 0
                i0 += 1
            else:
                (po, sz), priority = hi[i1], 1
                i1 += 1
            pltpu.make_async_copy(src.at[pl.ds(po, sz)], dst.at[pl.ds(po, sz)], sem).start(
                priority=priority)

    cx = pltpu.make_async_copy(x_h, x_v, sems.at[0])
    cb = pltpu.make_async_copy(b1_h, b1_v, sems.at[0])
    cx.start()
    cb.start()
    for n in range(NSEM):
        start_chunk(n)

    def wait_next():
        n = st["n"]
        src, dst, o, r, _ = chunks[n]
        whole = dst.at[pl.ds(o, r)]
        pltpu.make_async_copy(whole, whole, sems.at[n % NSEM]).wait()
        if n == 0:
            cx.wait()
            cb.wait()
        if n + NSEM < n_chunks:
            start_chunk(n + NSEM)
        st["n"] = n + 1

    wait_next()
    x = x_v[...].astype(F32)
    xn16 = _rows16(_ln(x)).astype(BF16)
    j16, par16 = _row_lane_ids()
    e2 = _expand_matrix()
    q = [jnp.zeros((16, D), F32) for _ in range(4)]
    for cc in range(4):
        lhs = _expand_masked(xn16[:, 128 * cc:128 * (cc + 1)], e2, j16, par16)
        for w in range(2):
            if cc + w > 0:
                wait_next()
        for g in range(4):
            rhs = jnp.concatenate([_head_pair(wq_v, cc, 4 * g + ii) for ii in range(4)], axis=0)
            q[g] = q[g] + jnp.dot(lhs, rhs, preferred_element_type=F32)
    j128 = lax.broadcasted_iota(jnp.int32, (16, 128), 0) % 8
    qm = []
    for g in range(4):
        qb = (q[g] * (D ** -0.5)).astype(BF16)
        qm.append(jnp.concatenate(
            [jnp.where(j128 // 2 == ii, qb, jnp.zeros_like(qb)) for ii in range(4)], axis=1))

    c_r = lax.broadcasted_iota(jnp.int32, (256, 128), 0)
    c_l = lax.broadcasted_iota(jnp.int32, (256, 128), 1)
    c2 = jnp.where(c_r // 2 == c_l, 1.0, 0.0).astype(BF16)
    qabs = [[None] * 4 for _ in range(4)]
    for cc in range(4):
        wait_next()
        wait_next()
        for g in range(4):
            rhs = jnp.concatenate([_head_pair(wuk_v, cc, 4 * g + ii) for ii in range(4)], axis=1)
            y = lax.dot_general(qm[g], rhs, NT, preferred_element_type=F32)
            y = jnp.where(par16 == j16 % 2, y, 0.0).astype(BF16)
            qabs[g][cc] = jnp.dot(y, c2, preferred_element_type=F32)
    qa = []
    for b in range(B):
        qa.append(jnp.concatenate(
            [jnp.concatenate([qabs[g][cc][8 * b:8 * b + 8] for cc in range(4)], axis=1)
             for g in range(4)], axis=0).astype(BF16))

    def scores(b, t, mrun):
        kv = ckv_v[pl.ds(b * SK + t * SUB, SUB), :]
        s = lax.dot_general(qa[b], kv, NT, preferred_element_type=F32)
        s_v[b, :, pl.ds(t * SUB, SUB)] = s
        for u in range(SUB // 128):
            mrun = jnp.maximum(mrun, s[:, 128 * u:128 * (u + 1)])
        return mrun

    def pv(b, t, m, acc, lrun):
        p = jnp.exp(s_v[b, :, pl.ds(t * SUB, SUB)] - m)
        for u in range(SUB // 128):
            lrun = lrun + p[:, 128 * u:128 * (u + 1)]
        kv = ckv_v[pl.ds(b * SK + t * SUB, SUB), :]
        return acc + jnp.dot(p.astype(BF16), kv, preferred_element_type=F32), lrun

    neg = jnp.full((H, 128), -jnp.inf, F32)
    mrun = neg
    for t in range(NS):
        wait_next()
        mrun = scores(0, t, mrun)
    m0 = jnp.max(mrun, axis=1, keepdims=True)
    mrun = neg
    acc, lrun = jnp.zeros((H, DC), F32), jnp.zeros((H, 128), F32)
    for t in range(NS):
        wait_next()
        mrun = scores(1, t, mrun)
        acc, lrun = pv(0, t, m0, acc, lrun)
    m1 = jnp.max(mrun, axis=1, keepdims=True)
    ctxc = [acc / jnp.sum(lrun, axis=1, keepdims=True)]
    acc, lrun = jnp.zeros((H, DC), F32), jnp.zeros((H, 128), F32)
    for t in range(NS):
        if t % 2 == 0:
            wait_next()
        acc, lrun = pv(1, t, m1, acc, lrun)
    ctxc.append(acc / jnp.sum(lrun, axis=1, keepdims=True))

    j16, par16 = _row_lane_ids()
    e2 = _expand_matrix()
    ctx = [jnp.zeros((16, D), F32) for _ in range(4)]
    cg = [jnp.concatenate([ctxc[0][8 * g:8 * g + 8], ctxc[1][8 * g:8 * g + 8]], axis=0).astype(BF16)
          for g in range(4)]
    for cc in range(4):
        lhs = [_expand_masked(cg[g][:, 128 * cc:128 * (cc + 1)], e2, j16, par16) for g in range(4)]
        for g in range(4):
            if g % 2 == 0:
                wait_next()
            rhs = jnp.concatenate([_head_pair(wuv_v, cc, 4 * g + ii) for ii in range(4)], axis=0)
            ctx[g] = ctx[g] + jnp.dot(lhs[g], rhs, preferred_element_type=F32)

    j128 = lax.broadcasted_iota(jnp.int32, (16, 128), 0) % 8
    acc = jnp.zeros((16, M), F32)
    for g in range(4):
        cbf = ctx[g].astype(BF16)
        lhs = jnp.concatenate(
            [jnp.where(j128 == j, cbf, jnp.zeros_like(cbf)) for j in range(8)], axis=1)
        wait_next()
        acc = acc + jnp.dot(lhs, wo_v[pl.ds(1024 * g, 1024), :], preferred_element_type=F32)
    att = jnp.concatenate([jnp.sum(acc[0:8], axis=0, keepdims=True),
                           jnp.sum(acc[8:16], axis=0, keepdims=True)], axis=0)
    h = x + att
    hn = _ln(h)
    r16 = lax.broadcasted_iota(jnp.int32, (16, M), 0)
    hn16 = jnp.where(r16 == 0, jnp.broadcast_to(hn[0:1], (16, M)),
                     jnp.where(r16 == 1, jnp.broadcast_to(hn[1:2], (16, M)), 0.0)).astype(BF16)

    t1 = jnp.zeros((8, F), F32)
    for kk in range(4):
        t1 = t1 + jnp.dot(hn16[:, 128 * kk:128 * (kk + 1)], w1_v[pl.ds(128 * kk, 128), :],
                          preferred_element_type=F32)[0:8]
    t1 = t1 + b1_v[...].reshape(1, F).astype(F32)
    sp = jnp.log1p(jnp.exp(-jnp.abs(t1))) + jnp.maximum(t1, 0.0)
    act = t1 * jnp.tanh(sp)
    act16 = jnp.concatenate([act, jnp.zeros((8, F), F32)], axis=0).astype(BF16)
    o = jnp.zeros((8, M), F32)
    off = 0
    for r in W2_CHUNKS:
        wait_next()
        o = o + jnp.dot(act16[:, off:off + r], w2_v[pl.ds(off, r), :],
                        preferred_element_type=F32)[0:8]
        off += r
    assert st["n"] == n_chunks
    out_ref[...] = (h + o[0:2]).astype(out_ref.dtype)


@jax.jit
def pallas_sequential_preLN__compressed_kv_cla__dense_activation_mish__decode_kernel(
    A_x: jax.Array,
    A_c_kv: jax.Array,
    A_w_q: jax.Array,
    A_w_uk: jax.Array,
    A_w_uv: jax.Array,
    A_w_o: jax.Array,
    B_x: jax.Array,
    B_w1: jax.Array,
    B_b1: jax.Array,
    B_w2: jax.Array,
):
    del B_x
    any_spec = pl.BlockSpec(memory_space=pl.ANY)
    out = pl.pallas_call(
        _kernel,
        out_shape=jax.ShapeDtypeStruct((B, M), A_x.dtype),
        in_specs=[any_spec] * 9,
        out_specs=pl.BlockSpec(memory_space=pltpu.VMEM),
        scratch_shapes=[
            pltpu.VMEM((B * SK, DC), BF16),
            pltpu.VMEM((M * H + PAD, D), BF16),
            pltpu.VMEM((DC * H + PAD, D), BF16),
            pltpu.VMEM((DC * H + PAD, D), BF16),
            pltpu.VMEM((H * D, M), BF16),
            pltpu.VMEM((M, F), BF16),
            pltpu.VMEM((F, M), BF16),
            pltpu.VMEM((B, H, SK), F32),
            pltpu.VMEM((B, M), BF16),
            pltpu.VMEM((F,), BF16),
            pltpu.SemaphoreType.DMA((NSEM,)),
        ],
        compiler_params=pltpu.CompilerParams(vmem_limit_bytes=64 * 1024 * 1024),
    )(A_x.reshape(B, M), B_b1, A_c_kv.reshape(B * SK, DC), A_w_q.reshape(M * H, D),
      A_w_uk.reshape(DC * H, D), A_w_uv.reshape(DC * H, D), A_w_o.reshape(H * D, M), B_w1, B_w2)
    return out.reshape(B, 1, M)
```
